```python
import jax
import jax.numpy as jnp

def _softmax(x, axis=-1):
    return jax.nn.softmax(x, axis=axis)
def _gelu(x):
    return jax.nn.gelu(x, approximate=True)
def _silu(x):
    return jax.nn.silu(x)
def _sigmoid(x):
    return jax.nn.sigmoid(x)
def _layernorm(x, axis=-1, eps=1e-5):
    m = jnp.mean(x, axis=axis, keepdims=True)
    v = jnp.var(x, axis=axis, keepdims=True)
    return (x - m) / jnp.sqrt(v + eps)
def _scatter_add(tgt, idx, src, axis=0):
    return tgt.at[idx].add(src)
def _segment_sum(src, seg, n):
    return jax.ops.segment_sum(src, seg, n)
class _Rng:
    def __init__(self, key):
        self._k = key
    def _next(self):
        self._k, sub = jax.random.split(self._k)
        return sub
    def normal(self, shape):
        return jax.random.normal(self._next(), shape, dtype=jnp.bfloat16)
    def randint(self, lo, hi, shape):
        return jax.random.randint(self._next(), shape, lo, hi, dtype=jnp.int32)
    def uniform(self, shape, lo=0.0, hi=1.0):
        return jax.random.uniform(self._next(), shape, jnp.bfloat16, lo, hi)
    def permutation(self, n):
        return jax.random.permutation(self._next(), n)


kernel_name = 'sequential_preLN__mha_block_cached__moe_arch_mod__decode'

def setup_inputs():
    _rng = _Rng(jax.random.key(int.from_bytes(__import__("os").urandom(4), "little")))
    _w = (lambda a: (lambda t: t.astype(jnp.bfloat16) if jnp.issubdtype(t.dtype, jnp.floating) else t)(jnp.asarray(a)))
    def _A_setup():
        B, Sq, D = 4, 1, 640
        H, Sk, Dh = 32, 8192, 192
        return {
            "x": _w((lambda *s: _rng.normal(s) * 0.05)(B, Sq, D)),
            "k_cache": _w((lambda *s: _rng.normal(s) * 0.05)(B, H, Sk, Dh)),
            "v_cache": _w((lambda *s: _rng.normal(s) * 0.05)(B, H, Sk, Dh)),
            "wq": _w((lambda *s: _rng.normal(s) * 0.05)(D, H * Dh) * (D ** -0.5)),
            "wo": _w((lambda *s: _rng.normal(s) * 0.05)(H * Dh, D) * ((H * Dh) ** -0.5)),
        }
    _A_in = _A_setup()

    def _B_setup():
        B, S, D, F, C = 4, 1, 640, 1536, 1
        return {
            "x": _w((lambda *s: _rng.normal(s) * 0.05)(B, S, D)),
            "w_r": _w((lambda *s: _rng.normal(s) * 0.05)(D)),
            "w_gate": _w((lambda *s: _rng.normal(s) * 0.05)(D, F)),
            "w_up": _w((lambda *s: _rng.normal(s) * 0.05)(D, F)),
            "w_down": _w((lambda *s: _rng.normal(s) * 0.05)(F, D)),
        }
    _B_in = _B_setup()

    return {
        "A_x": _A_in["x"],
        "A_k_cache": _A_in["k_cache"],
        "A_v_cache": _A_in["v_cache"],
        "A_wq": _A_in["wq"],
        "A_wo": _A_in["wo"],
        "B_x": _B_in["x"],
        "B_w_r": _B_in["w_r"],
        "B_w_gate": _B_in["w_gate"],
        "B_w_up": _B_in["w_up"],
        "B_w_down": _B_in["w_down"],
    }

def reference(A_x, A_k_cache, A_v_cache, A_wq, A_wo, B_x, B_w_r, B_w_gate, B_w_up, B_w_down):
    def _A_ref(x, k_cache, v_cache, wq, wo):
        B, Sq, D = x.shape
        H, Dh = 32, 192
        q = (lambda x, *d: x.transpose(*d))((x @ wq).reshape(B, Sq, H, Dh), 0, 2, 1, 3)
        scores = jnp.einsum("bhqd,bhkd->bhqk", q, k_cache) * (Dh ** -0.5)
        p = _softmax(scores, axis=-1)
        o = jnp.einsum("bhqk,bhkd->bhqd", p, v_cache)
        return (lambda x, *d: x.transpose(*d))(o, 0, 2, 1, 3).reshape(B, Sq, H * Dh) @ wo

    def _B_ref(x, w_r, w_gate, w_up, w_down):
        B, S, D = x.shape
        C = 1
        r = x @ w_r
        idx = jnp.argsort(-r, axis=-1)[:, :C]
        idx_e = jnp.repeat(idx.reshape(B, C, 1), D, axis=2)
        x_sel = jnp.take_along_axis(x, idx_e, axis=1)
        g = _silu(x_sel @ w_gate)
        u = x_sel @ w_up
        y = (g * u) @ w_down
        r_sel = _sigmoid(jnp.take_along_axis(r, idx, axis=1))
        y = y * r_sel.reshape(B, C, 1)
        b_off = (jnp.arange(B) * S).reshape(B, 1)
        flat_idx = (idx + b_off).reshape(B * C)
        zero = (x * 0.0).reshape(B * S, D)
        upd = _scatter_add(zero, flat_idx, y.reshape(B * C, D), axis=0)
        return x + upd.reshape(B, S, D)

    x = A_x
    h = x + _A_ref(_layernorm(x, axis=-1), A_k_cache, A_v_cache, A_wq, A_wo)
    h2 = h + _B_ref(_layernorm(h, axis=-1), B_w_r, B_w_gate, B_w_up, B_w_down)
    return h2
```

```python
import jax
import jax.numpy as jnp
from jax import lax
from jax.experimental import pallas as pl
from jax.experimental.pallas import tpu as pltpu

B, D, H, SK, DH, F = 4, 640, 32, 8192, 192, 1536
CW = 256
NC = SK // CW
NG = NC // 2
NB = 3 * NC
NHEAD = B * H
EPS = 1e-5
f32 = jnp.float32
bf16 = jnp.bfloat16


def _ln(x):
    m = jnp.mean(x, axis=-1, keepdims=True)
    c = x - m
    v = jnp.mean(c * c, axis=-1, keepdims=True)
    return c / jnp.sqrt(v + EPS)


def _kernel(x_hbm, k_hbm, v_hbm, wq_hbm, wo_hbm, wr_hbm, wg_hbm, wu_hbm, wd_hbm, o_ref,
         ring, x_v, wr_v, wq_v, wo_v, wg_v, wu_v, wd_v, q_s, s_s, out_s,
         rsem, ssem, qsem, osem, gsem, dsem):
    def kv_copy(src, head, c, slot):
        return pltpu.make_async_copy(
            src.at[pl.ds(pl.multiple_of(head * DH, DH), DH), pl.ds(pl.multiple_of(c * CW, CW), CW)],
            ring.at[slot], rsem.at[slot])

    def kv_start(src, head, g, slot):
        kv_copy(src, head, 2 * g, slot).start(priority=0)
        kv_copy(src, head, 2 * g + 1, slot + 1).start(priority=1)

    def slot_wait(slot):
        pltpu.make_async_copy(ring.at[slot], ring.at[slot], rsem.at[slot]).wait()

    x_cp = pltpu.make_async_copy(x_hbm, x_v, ssem.at[0])
    wr_cp = pltpu.make_async_copy(wr_hbm, wr_v, ssem.at[1])
    x_cp.start()

    def wq_pair(i, _):
        r = pl.multiple_of((i % 5) * 128, 128)
        j = (i // 5) * 2
        for p in range(2):
            pltpu.make_async_copy(
                wq_hbm.at[pl.ds(r, 128), pl.ds(pl.multiple_of((j + p) * 384, 384), 384)],
                wq_v.at[j + p, pl.ds(r, 128)], qsem.at[j + p]).start(priority=p)
        return 0
    lax.fori_loop(0, 40, wq_pair, 0)
    wr_cp.start()

    x_cp.wait()
    x = x_v[...].astype(f32)
    xn = _ln(x)
    xn8 = jnp.concatenate([xn, jnp.zeros((12, D), f32)], axis=0).astype(bf16)

    def q_step(j, _):
        for t in range(5):
            i = j * 5 + t
            pltpu.make_async_copy(
                wo_hbm.at[pl.ds(pl.multiple_of(j * 384, 384), 384), pl.ds(t * 128, 128)],
                wo_v.at[pl.ds(pl.multiple_of(j * 384, 384), 384), pl.ds(t * 128, 128)],
                osem.at[0]).start(priority=t % 2)
        pltpu.make_async_copy(wq_v.at[j], wq_v.at[j], qsem.at[j]).wait()
        q = jnp.dot(xn8, wq_v[j], preferred_element_type=f32)[:8]
        q_s[j] = q * (DH ** -0.5)
        return 0
    lax.fori_loop(0, 16, q_step, 0)

    def first(g, _):
        kv_start(k_hbm, 0, g, 2 * g)
        return 0
    lax.fori_loop(0, NG, first, 0)

    def second(g, _):
        kv_start(v_hbm, 0, g, NC + 2 * g)
        return 0
    lax.fori_loop(0, NG, second, 0)

    def third(g, _):
        kv_start(k_hbm, 1, g, 2 * NC + 2 * g)
        return 0
    lax.fori_loop(0, NG, third, 0)

    out_s[...] = jnp.zeros_like(out_s)
    pltpu.make_async_copy(wo_v, wo_v, osem.at[0]).wait()

    def ffn_start(i):
        @pl.when(i < 20)
        def _():
            j = i // 5
            r = pl.multiple_of((i % 5) * 128, 128)
            for p, (src, dst) in enumerate(((wg_hbm, wg_v), (wu_hbm, wu_v))):
                pltpu.make_async_copy(
                    src.at[pl.ds(r, 128), pl.ds(pl.multiple_of(j * 384, 384), 384)],
                    dst.at[j, pl.ds(r, 128)], gsem.at[j]).start(priority=p)

        @pl.when(jnp.logical_and(i >= 20, i < 30))
        def _():
            j = (i - 20) // 2
            for p in range(2):
                r = pl.multiple_of((((i - 20) % 2) * 2 + p) * 384, 384)
                pltpu.make_async_copy(
                    wd_hbm.at[pl.ds(r, 384), pl.ds(pl.multiple_of(j * 128, 128), 128)],
                    wd_v.at[j, pl.ds(r, 384)], dsem.at[j]).start(priority=p)

    def head_body(i, base):
        b = i // H
        h = i % H
        kbase = base
        vbase = jnp.where(base == 2 * NC, 0, base + NC)
        nbase = jnp.where(vbase == 2 * NC, 0, vbase + NC)

        qrow = q_s[h // 2, pl.ds(b, 1), :]
        qt = jnp.transpose(jnp.broadcast_to(qrow, (128, 384)))
        qb = jnp.where(h % 2 == 0, qt[:DH], qt[DH:])

        def k_step(g, m):
            slot = kbase + 2 * g
            for p in range(2):
                slot_wait(slot + p)
            for p in range(2):
                for t in range(2):
                    kt = ring[slot + p, :, t * 128:(t + 1) * 128].astype(f32)
                    s = jnp.sum((kt * qb).reshape(DH // 8, 8, 128), axis=0)
                    s = jnp.broadcast_to(jnp.sum(s, axis=0, keepdims=True), (8, 128))
                    s_s[g * 4 + p * 2 + t] = s
                    m = jnp.maximum(m, s)

            @pl.when(i < NHEAD - 1)
            def _():
                kv_start(v_hbm, i + 1, g, slot)

            @pl.when(i == NHEAD - 1)
            def _():
                ffn_start(NG + g)
            return m
        m = lax.fori_loop(0, NG, k_step, jnp.full((8, 128), -jnp.inf, f32))
        m = jnp.broadcast_to(jnp.max(m, axis=1, keepdims=True), (8, 128))

        def v_step(g, carry):
            acc, l = carry
            slot = vbase + 2 * g
            for p in range(2):
                slot_wait(slot + p)
            for p in range(2):
                for t in range(2):
                    e = jnp.exp(s_s[g * 4 + p * 2 + t] - m)
                    l = l + e
                    vt = ring[slot + p, :, t * 128:(t + 1) * 128].astype(f32)
                    acc = acc + vt.reshape(DH // 8, 8, 128) * e

            @pl.when(i < NHEAD - 2)
            def _():
                kv_start(k_hbm, i + 2, g, slot)

            @pl.when(i == NHEAD - 2)
            def _():
                ffn_start(g)
            return acc, l
        acc, l = lax.fori_loop(0, NG, v_step,
                               (jnp.zeros((DH // 8, 8, 128), f32), jnp.zeros((8, 128), f32)))
        lsum = jnp.sum(l, axis=1, keepdims=True)
        o = jnp.sum(acc, axis=2, keepdims=True) / lsum
        w = wo_v[pl.ds(pl.multiple_of(h * DH, DH), DH), :].astype(f32).reshape(DH // 8, 8, D)
        out_s[b] += jnp.sum(w * o, axis=0)
        return nbase
    lax.fori_loop(0, NHEAD, head_body, jnp.int32(0))

    attn = jnp.concatenate([jnp.sum(out_s[b], axis=0, keepdims=True) for b in range(B)], axis=0)
    hid = x + attn
    hn = _ln(hid)
    hn16 = jnp.concatenate([hn, jnp.zeros((12, D), f32)], axis=0).astype(bf16)
    wr_cp.wait()
    r = jnp.sum(hn * wr_v[...].astype(f32).reshape(1, D), axis=-1, keepdims=True)
    acts = []
    for j in range(4):
        pltpu.make_async_copy(wg_v.at[j], wg_v.at[j], gsem.at[j]).wait()
        pltpu.make_async_copy(wu_v.at[j], wu_v.at[j], gsem.at[j]).wait()
        g = jnp.dot(hn16, wg_v[j], preferred_element_type=f32)
        u = jnp.dot(hn16, wu_v[j], preferred_element_type=f32)
        acts.append((g * jax.nn.sigmoid(g) * u).astype(bf16))
    a = jnp.concatenate(acts, axis=1)
    ys = []
    for j in range(5):
        pltpu.make_async_copy(wd_v.at[j], wd_v.at[j], dsem.at[j]).wait()
        ys.append(jnp.dot(a, wd_v[j], preferred_element_type=f32)[:B])
    y = jnp.concatenate(ys, axis=1) * jax.nn.sigmoid(r)
    o_ref[...] = (hid + (hn + (hn * 0.0 + y))).astype(o_ref.dtype)

@jax.jit
def pallas_sequential_preLN__mha_block_cached__moe_arch_mod__decode_kernel(A_x, A_k_cache, A_v_cache, A_wq, A_wo, B_x, B_w_r, B_w_gate, B_w_up, B_w_down):
    kt = jnp.transpose(A_k_cache, (0, 1, 3, 2)).reshape(B * H * DH, SK)
    vt = jnp.transpose(A_v_cache, (0, 1, 3, 2)).reshape(B * H * DH, SK)
    out = pl.pallas_call(
        _kernel,
        in_specs=[pl.BlockSpec(memory_space=pl.ANY)] * 9,
        out_specs=pl.BlockSpec(memory_space=pltpu.VMEM),
        out_shape=jax.ShapeDtypeStruct((B, D), A_x.dtype),
        scratch_shapes=[
            pltpu.VMEM((NB, DH, CW), bf16),
            pltpu.VMEM((B, D), bf16),
            pltpu.VMEM((D,), bf16),
            pltpu.VMEM((16, D, 384), bf16),
            pltpu.VMEM((H * DH, D), bf16),
            pltpu.VMEM((4, D, 384), bf16),
            pltpu.VMEM((4, D, 384), bf16),
            pltpu.VMEM((5, F, 128), bf16),
            pltpu.VMEM((16, 8, 384), f32),
            pltpu.VMEM((SK // 128, 8, 128), f32),
            pltpu.VMEM((B, 8, D), f32),
            pltpu.SemaphoreType.DMA((NB,)),
            pltpu.SemaphoreType.DMA((2,)),
            pltpu.SemaphoreType.DMA((16,)),
            pltpu.SemaphoreType.DMA((1,)),
            pltpu.SemaphoreType.DMA((4,)),
            pltpu.SemaphoreType.DMA((5,)),
        ],
        compiler_params=pltpu.CompilerParams(vmem_limit_bytes=64 * 1024 * 1024, disable_bounds_checks=True),
    )(A_x.reshape(B, D), kt, vt, A_wq, A_wo, B_w_r, B_w_gate, B_w_up, B_w_down)
    return out.reshape(B, 1, D)
```

```python
import jax
import jax.numpy as jnp
from jax import lax
from jax.experimental import pallas as pl
from jax.experimental.pallas import tpu as pltpu

B, D, H, SK, DH, F = 4, 640, 32, 8192, 192, 1536
EPS = 1e-5
CW = 256
NG = SK // (2 * CW)
NSLOT = 3 * NG
NHEAD = B * H
QW = 4 * DH
FW = 384
DOWN_GROUPS = ((0, 384), (384, 384), (768, 384), (1152, 256), (1408, 128))
f32 = jnp.float32
bf16 = jnp.bfloat16


def _layernorm(x):
    c = x - jnp.mean(x, axis=-1, keepdims=True)
    v = jnp.mean(c * c, axis=-1, keepdims=True)
    return c / jnp.sqrt(v + EPS)


def _mxu_rows(x):
    return jnp.concatenate([x, jnp.zeros((16 - B, D), f32)], axis=0).astype(bf16)


def _wait_filled(buf, sem):
    pltpu.make_async_copy(buf, buf, sem).wait()


def _kernel(x_hbm, k_hbm, v_hbm, wq_hbm, wo_hbm, wr_hbm, wg_hbm, wu_hbm, wd_hbm, o_ref,
            ring, x_v, wr_v, wq_v, wo_v, wgu_v, wd_v, q_s, s_s, attn_s, gu_sem, d_sem):

    def ffn_start(t):
        @pl.when(t < 20)
        def _():
            j = t // 5
            rows = pl.ds(pl.multiple_of((t % 5) * 128, 128), 128)
            cols = pl.ds(pl.multiple_of(j * FW, FW), FW)
            for p, src in enumerate((wg_hbm, wu_hbm)):
                pltpu.make_async_copy(
                    src.at[rows, cols], wgu_v.at[j, p, rows], gu_sem.at[j]).start(priority=p)

        @pl.when(t >= 20)
        def _():
            u = t - 20
            grp = jnp.where(u == 11, 4, u // 3)
            for p in range(2):
                rows = pl.ds(pl.multiple_of(u * 128 + p * 64, 64), 64)
                pltpu.make_async_copy(
                    wd_hbm.at[rows], wd_v.at[rows], d_sem.at[grp]).start(priority=p)

    def attention(ring_sem, q_sem, sem):
        def kv_start(src, head, g, slot):
            rows = pl.ds(pl.multiple_of(head * DH, DH), DH)
            for p in range(2):
                cols = pl.ds(pl.multiple_of((2 * g + p) * CW, CW), CW)
                pltpu.make_async_copy(
                    src.at[rows, cols], ring.at[slot, p], ring_sem.at[slot]).start(priority=p)

        x_cp = pltpu.make_async_copy(x_hbm, x_v, sem.at[0])
        wr_cp = pltpu.make_async_copy(wr_hbm, wr_v, sem.at[1])
        x_cp.start()
        wr_cp.start(priority=1)

        def wq_start(j, carry):
            for t in range(9):
                rows, u = pl.ds((t // 3) * 192, 192), t % 3
                pltpu.make_async_copy(
                    wq_hbm.at[rows, pl.ds(pl.multiple_of(j * QW + u * 256, 256), 256)],
                    wq_v.at[j, rows, pl.ds(u * 256, 256)], q_sem.at[j]).start(priority=t % 2)
            pltpu.make_async_copy(
                wq_hbm.at[pl.ds(576, 64), pl.ds(pl.multiple_of(j * QW, QW), QW)],
                wq_v.at[j, pl.ds(576, 64)], q_sem.at[j]).start(priority=1)
            return carry
        lax.fori_loop(0, H // 4, wq_start, 0)

        x_cp.wait()
        xn = _mxu_rows(_layernorm(x_v[...].astype(f32)))

        def q_step(j, carry):
            for u in range(2):
                r0 = 0
                for t, n in enumerate((80, 80, 80, 72, 72)):
                    rows = pl.ds(pl.multiple_of(j * QW + u * 2 * DH + r0, 8), n)
                    pltpu.make_async_copy(
                        wo_hbm.at[rows], wo_v.at[rows], sem.at[2]).start(priority=(t + u) % 2)
                    r0 += n
                if u == 0:
                    _wait_filled(wq_v.at[j], q_sem.at[j])
                q = jnp.dot(xn, wq_v[j, :, u * 2 * DH:(u + 1) * 2 * DH],
                            preferred_element_type=f32)
                q_s[2 * j + u] = q[:8] * (DH ** -0.5)
            return carry
        lax.fori_loop(0, H // 4, q_step, 0)

        for third, (src, head) in enumerate(((k_hbm, 0), (v_hbm, 0), (k_hbm, 1))):
            def fill(g, carry, src=src, head=head, third=third):
                kv_start(src, head, g, third * NG + g)
                return carry
            lax.fori_loop(0, NG, fill, 0)

        attn_s[...] = jnp.zeros((B, 8, D), f32)
        _wait_filled(wo_v, sem.at[2])
        wr_cp.wait()

        def head_step(i, kbase):
            b = i // H
            h = i % H
            vbase = jnp.where(kbase == 2 * NG, 0, kbase + NG)

            qrow = q_s[h // 2, pl.ds(b, 1), :]
            qt = jnp.transpose(jnp.broadcast_to(qrow, (128, 2 * DH)))
            qb = jnp.where(h % 2 == 0, qt[:DH], qt[DH:])

            def k_step(g, m):
                slot = kbase + g
                _wait_filled(ring.at[slot], ring_sem.at[slot])
                for p in range(2):
                    for t in range(2):
                        kt = ring[slot, p, :, t * 128:(t + 1) * 128].astype(f32)
                        s = jnp.sum((kt * qb).reshape(DH // 8, 8, 128), axis=0)
                        s = jnp.broadcast_to(jnp.sum(s, axis=0, keepdims=True), (8, 128))
                        s_s[g * 4 + p * 2 + t] = s
                        m = jnp.maximum(m, s)

                @pl.when(i < NHEAD - 1)
                def _():
                    kv_start(v_hbm, i + 1, g, slot)

                @pl.when(i == NHEAD - 1)
                def _():
                    ffn_start(NG + g)
                return m
            m = lax.fori_loop(0, NG, k_step, jnp.full((8, 128), -jnp.inf, f32))
            m = jnp.broadcast_to(jnp.max(m, axis=1, keepdims=True), (8, 128))

            def v_step(g, carry):
                acc, l = carry
                slot = vbase + g
                _wait_filled(ring.at[slot], ring_sem.at[slot])
                for p in range(2):
                    for t in range(2):
                        e = jnp.exp(s_s[g * 4 + p * 2 + t] - m)
                        l = l + e
                        vt = ring[slot, p, :, t * 128:(t + 1) * 128].astype(f32)
                        acc = acc + vt.reshape(DH // 8, 8, 128) * e

                @pl.when(i < NHEAD - 2)
                def _():
                    kv_start(k_hbm, i + 2, g, slot)

                @pl.when(i == NHEAD - 2)
                def _():
                    ffn_start(g)
                return acc, l
            acc, l = lax.fori_loop(
                0, NG, v_step, (jnp.zeros((DH // 8, 8, 128), f32), jnp.zeros((8, 128), f32)))

            o = jnp.sum(acc, axis=2, keepdims=True) / jnp.sum(l, axis=1, keepdims=True)
            w = wo_v[pl.ds(pl.multiple_of(h * DH, DH), DH), :].astype(f32)
            attn_s[b] += jnp.sum(w.reshape(DH // 8, 8, D) * o, axis=0)
            return jnp.where(vbase == 2 * NG, 0, vbase + NG)
        lax.fori_loop(0, NHEAD, head_step, jnp.int32(0))

    pl.run_scoped(attention,
                  pltpu.SemaphoreType.DMA((NSLOT,)),
                  pltpu.SemaphoreType.DMA((H // 4,)),
                  pltpu.SemaphoreType.DMA((3,)))

    attn = jnp.concatenate(
        [jnp.sum(attn_s[b], axis=0, keepdims=True) for b in range(B)], axis=0)
    hid = x_v[...].astype(f32) + attn
    hn = _layernorm(hid)

    r = jnp.sum(hn * wr_v[...].astype(f32).reshape(1, D), axis=-1, keepdims=True)
    gate = jax.nn.sigmoid(r)
    hn16 = _mxu_rows(hn)
    acts = []
    for j in range(F // FW):
        _wait_filled(wgu_v.at[j], gu_sem.at[j])
        g = jnp.dot(hn16, wgu_v[j, 0], preferred_element_type=f32)
        u = jnp.dot(hn16, wgu_v[j, 1], preferred_element_type=f32)
        acts.append((g * jax.nn.sigmoid(g) * u).astype(bf16))
    act = jnp.concatenate(acts, axis=1)
    y = jnp.zeros((B, D), f32)
    for j, (r0, n) in enumerate(DOWN_GROUPS):
        _wait_filled(wd_v.at[pl.ds(r0, n)], d_sem.at[j])
        y = y + jnp.dot(act[:, r0:r0 + n], wd_v[pl.ds(r0, n), :], preferred_element_type=f32)[:B]
    o_ref[...] = (hid + (hn + (hn * 0.0 + y * gate))).astype(o_ref.dtype)


@jax.jit
def pallas_sequential_preLN__mha_block_cached__moe_arch_mod__decode_kernel(
    A_x: jax.Array,
    A_k_cache: jax.Array,
    A_v_cache: jax.Array,
    A_wq: jax.Array,
    A_wo: jax.Array,
    B_x: jax.Array,
    B_w_r: jax.Array,
    B_w_gate: jax.Array,
    B_w_up: jax.Array,
    B_w_down: jax.Array,
):
    del B_x
    kt = jnp.transpose(A_k_cache, (0, 1, 3, 2)).reshape(B * H * DH, SK)
    vt = jnp.transpose(A_v_cache, (0, 1, 3, 2)).reshape(B * H * DH, SK)
    out = pl.pallas_call(
        _kernel,
        in_specs=[pl.BlockSpec(memory_space=pl.ANY)] * 9,
        out_specs=pl.BlockSpec(memory_space=pltpu.VMEM),
        out_shape=jax.ShapeDtypeStruct((B, D), A_x.dtype),
        scratch_shapes=[
            pltpu.VMEM((NSLOT, 2, DH, CW), bf16),
            pltpu.VMEM((B, D), bf16),
            pltpu.VMEM((D,), bf16),
            pltpu.VMEM((H // 4, D, QW), bf16),
            pltpu.VMEM((H * DH, D), bf16),
            pltpu.VMEM((F // FW, 2, D, FW), bf16),
            pltpu.VMEM((F, D), bf16),
            pltpu.VMEM((H // 2, 8, 2 * DH), f32),
            pltpu.VMEM((SK // 128, 8, 128), f32),
            pltpu.VMEM((B, 8, D), f32),
            pltpu.SemaphoreType.DMA((F // FW,)),
            pltpu.SemaphoreType.DMA((len(DOWN_GROUPS),)),
        ],
        compiler_params=pltpu.CompilerParams(vmem_limit_bytes=48 * 1024 * 1024),
    )(A_x.reshape(B, D), kt, vt, A_wq, A_wo, B_w_r, B_w_gate, B_w_up, B_w_down)
    return out.reshape(B, 1, D)
```
